```python
import os as _os
_os.environ.setdefault('JAX_PLATFORMS', 'cpu')
import jax
import jax.numpy as jnp

def _softmax(x, axis=-1):
    return jax.nn.softmax(x, axis=axis)

def _gelu(x):
    return jax.nn.gelu(x, approximate=True)

def _silu(x):
    return jax.nn.silu(x)

def _sigmoid(x):
    return jax.nn.sigmoid(x)

def _layernorm(x, axis=-1, eps=1e-05):
    m = jnp.mean(x, axis=axis, keepdims=True)
    v = jnp.var(x, axis=axis, keepdims=True)
    return (x - m) / jnp.sqrt(v + eps)

def _scatter_add(tgt, idx, src, axis=0):
    return tgt.at[idx].add(src)

def _segment_sum(src, seg, n):
    return jax.ops.segment_sum(src, seg, n)

class _Rng:

    def __init__(self, key):
        self._k = key

    def _next(self):
        self._k, sub = jax.random.split(self._k)
        return sub

    def normal(self, shape):
        return jax.random.normal(self._next(), shape, dtype=jnp.bfloat16)

    def randint(self, lo, hi, shape):
        return jax.random.randint(self._next(), shape, lo, hi, dtype=jnp.int32)

    def uniform(self, shape, lo=0.0, hi=1.0):
        return jax.random.uniform(self._next(), shape, jnp.bfloat16, lo, hi)

    def permutation(self, n):
        return jax.random.permutation(self._next(), n)
kernel_name = 'standalone__conformer_conv_module__speech'

def setup_inputs():
    _rng = _Rng(jax.random.key(int.from_bytes(__import__("os").urandom(4), "little")))
    _w = lambda a: (lambda t: t.astype(jnp.bfloat16) if jnp.issubdtype(t.dtype, jnp.floating) else t)(jnp.asarray(a))
    B, T, D, K = (2, 16000, 256, 5)
    return {'x': _w((lambda *s: _rng.normal(s) * 0.2)(B, T, D)), 'w_pw1': _w((lambda *s: _rng.normal(s) * 0.2)(D, 2 * D)), 'dw': _w((lambda *s: _rng.normal(s) * 0.05)(K, D)), 'w_pw2': _w((lambda *s: _rng.normal(s) * 0.05)(D, D))}

def reference(x, w_pw1, dw, w_pw2):
    B, T, D = x.shape
    K = dw.shape[0]
    h = x @ w_pw1
    a, b = (h[..., :D].copy(), h[..., D:].copy())
    h = a * _sigmoid(b)
    pad = K // 2
    hp = jnp.pad(h, ((0, 0), (pad, pad), (0, 0)))
    out = jnp.zeros_like(h)
    for i in range(K):
        out = out + hp[:, i:i + T, :] * dw[i][None, None, :]
    return _silu(out) @ w_pw2
```

```python
import functools
import jax
import jax.numpy as jnp
from jax.experimental import pallas as pl
from jax.experimental.pallas import tpu as pltpu


def _kernel(xp_ref, x_ref, xn_ref, w1_ref, dw_ref, w2_ref, o_ref, h_ref, *, M, D, K, nT):
    t = pl.program_id(1)
    pad = K // 2
    w1 = w1_ref[...]

    def glu(xv):
        h = jnp.dot(xv, w1, preferred_element_type=jnp.float32)
        a = h[:, :D]
        b = h[:, D:]
        return a * (0.5 * jnp.tanh(0.5 * b) + 0.5)

    hm = glu(x_ref[...])
    hp = glu(xp_ref[...])
    hn = glu(xn_ref[...])
    hp = jnp.where(t > 0, hp, 0.0)
    hn = jnp.where(t < nT - 1, hn, 0.0)
    for c in range(D // 128):
        h_ref[c, 0:16, :] = hp[:, c * 128:(c + 1) * 128]
        h_ref[c, 16:16 + M, :] = hm[:, c * 128:(c + 1) * 128]
        h_ref[c, 16 + M:32 + M, :] = hn[:, c * 128:(c + 1) * 128]
    dw = dw_ref[...].astype(jnp.float32)
    outs = []
    for c in range(D // 128):
        acc = None
        for k in range(K):
            term = h_ref[c, 16 - pad + k:16 - pad + k + M, :] * dw[k:k + 1, c * 128:(c + 1) * 128]
            acc = term if acc is None else acc + term
        y = acc * (0.5 * jnp.tanh(0.5 * acc) + 0.5)
        outs.append(y.astype(jnp.bfloat16))
    y = jnp.concatenate(outs, axis=1)
    o_ref[...] = jnp.dot(y, w2_ref[...], preferred_element_type=jnp.float32).astype(o_ref.dtype)


@jax.jit
def pallas_standalone__conformer_conv_module__speech_kernel(x, w_pw1, dw, w_pw2):
    M = 1600
    if True:
        B, T, D = x.shape
        K = dw.shape[0]
        nT = T // M
        r = M // 16
        n16 = T // 16
        return pl.pallas_call(
            functools.partial(_kernel, M=M, D=D, K=K, nT=nT),
            grid=(B, nT),
            in_specs=[
                pl.BlockSpec((None, 16, D), lambda b, t: (b, jnp.maximum(t * r - 1, 0), 0)),
                pl.BlockSpec((None, M, D), lambda b, t: (b, t, 0)),
                pl.BlockSpec((None, 16, D), lambda b, t: (b, jnp.minimum((t + 1) * r, n16 - 1), 0)),
                pl.BlockSpec((D, 2 * D), lambda b, t: (0, 0)),
                pl.BlockSpec((K, D), lambda b, t: (0, 0)),
                pl.BlockSpec((D, D), lambda b, t: (0, 0)),
            ],
            out_specs=pl.BlockSpec((None, M, D), lambda b, t: (b, t, 0)),
            out_shape=jax.ShapeDtypeStruct((B, T, D), x.dtype),
            scratch_shapes=[pltpu.VMEM((D // 128, M + 32, 128), jnp.float32)],
            compiler_params=pltpu.CompilerParams(
                dimension_semantics=("parallel", "parallel"),
                vmem_limit_bytes=100 * 1024 * 1024),
        )(x, x, x, w_pw1, dw, w_pw2)
```

```python
import functools

import jax
import jax.numpy as jnp
from jax import lax
from jax.experimental import pallas as pl
from jax.experimental.pallas import tpu as pltpu

F32 = jnp.float32
LANES = 128
NEG_LOG2_E = -1.4426950408889634
PAD_ROWS = 8
LOOKAHEAD = 2
MAX_SUB_ROWS = 320
RAMP = (1, 2, 5, 15)


def _schedule(n_rows_per_batch, batch):
  r = max((c for c in range(16, MAX_SUB_ROWS + 1, 16)
           if n_rows_per_batch % c == 0),
          default=None)
  if r is None:
    raise ValueError("sequence length must be a multiple of 16")
  n_sub = batch * n_rows_per_batch // r
  pre = []
  for c in RAMP:
    if sum(pre) + c < n_sub:
      pre.append(c)
  if not pre:
    raise ValueError("problem too small")
  n_mid = n_sub - sum(pre) - 1
  per_iter = n_mid // 2
  n_iter = 2 if per_iter else 0
  post = n_mid - per_iter * n_iter + 1
  fine = 2 if r % 32 == 0 else 1
  return r, tuple(pre), per_iter, n_iter, post, fine


def _sigmoid(z):
  return pltpu.reciprocal(1.0 + jnp.exp2(z * NEG_LOG2_E), approx=True)


def _conformer_conv_kernel(
    x_hbm, w1_hbm, dw_hbm, w2_hbm, o_hbm,
    xbuf, obuf, hbuf, w1_vmem, dw_raw, dw_f32, w2_vmem,
    x_sem, o_sem, w_sem,
    *, batch, seq, dim, taps, rows, pre, per_iter, n_iter, post, fine):
  pad = taps // 2
  n_col = dim // LANES
  sub_per_seq = seq // rows
  n_sub = batch * sub_per_seq
  loop_start = sum(pre)

  chunks, j = [], 0
  for cnt in (*pre, *([per_iter] * n_iter), post):
    chunks.append((j, cnt))
    j += cnt
  assert j == n_sub
  n_pre, n_chunks = len(pre), len(chunks)

  def aligned(i, m):
    return i if isinstance(i, int) else pl.multiple_of(i, m)

  def x_copy(c, first_sub, cnt):
    sl = pl.ds(aligned(first_sub * rows, rows), cnt * rows)
    return pltpu.make_async_copy(x_hbm.at[sl, :], xbuf.at[sl, :], x_sem.at[c])

  def x_chunk(c):
    return x_copy(c, *chunks[c])

  def out_copy(start_row, n_rows):
    sl = pl.ds(aligned(start_row, PAD_ROWS), n_rows)
    return pltpu.make_async_copy(obuf.at[sl, :], o_hbm.at[sl, :], o_sem.at[0])

  w1_copy = pltpu.make_async_copy(w1_hbm, w1_vmem, w_sem.at[0])
  dw_copy = pltpu.make_async_copy(dw_hbm, dw_raw, w_sem.at[1])
  w2_copy = pltpu.make_async_copy(w2_hbm, w2_vmem, w_sem.at[2])
  x_chunk(0).start(priority=0)
  w1_copy.start(priority=0)
  dw_copy.start(priority=1)
  w2_copy.start(priority=1)
  for c in range(1, min(LOOKAHEAD, n_chunks)):
    x_chunk(c).start(priority=1)

  zeros = jnp.zeros((PAD_ROWS, LANES), F32)
  for c in range(n_col):
    hbuf[c, pl.ds(0, PAD_ROWS), :] = zeros
    hbuf[c, pl.ds(PAD_ROWS + batch * seq, PAD_ROWS), :] = zeros
  row_iota = lax.broadcasted_iota(jnp.int32, (8, LANES), 0)

  def p1(base, off, n=rows):
    xv = xbuf[pl.ds(aligned(base + off, 16), n), :]
    ab = jnp.dot(xv, w1_vmem[...], preferred_element_type=F32)
    h = ab[:, :dim] * _sigmoid(ab[:, dim:])
    for c in range(n_col):
      hbuf[c, pl.ds(aligned(base + (PAD_ROWS + off), 8), n), :] = (
          h[:, c * LANES:(c + 1) * LANES])

  def p2(base, off, n, is_first, is_last):
    masks = {}
    for k in range(taps):
      if k < pad and is_first is not False:
        lim = pad - k
        if is_first is not True:
          lim = jnp.where(is_first, lim, 0)
        masks[k] = row_iota < lim
      if k > pad and is_last is not False:
        lim = 8 - (k - pad)
        if is_last is not True:
          lim = jnp.where(is_last, lim, 8)
        masks[k] = row_iota >= lim
    cols = []
    for c in range(n_col):
      acc = None
      for k in range(taps):
        v = hbuf[c, pl.ds(base + (PAD_ROWS + off + k - pad), n), :]
        if k in masks and k < pad:
          v = jnp.concatenate([jnp.where(masks[k], 0.0, v[:8]), v[8:]], axis=0)
        elif k in masks:
          v = jnp.concatenate(
              [v[:n - 8], jnp.where(masks[k], 0.0, v[n - 8:])], axis=0)
        term = v * dw_f32[k:k + 1, c * LANES:(c + 1) * LANES]
        acc = term if acc is None else acc + term
      cols.append(acc * _sigmoid(acc))
    y = jnp.concatenate(cols, axis=1).astype(w2_vmem.dtype)
    out = jnp.dot(y, w2_vmem[...], preferred_element_type=F32)
    obuf[pl.ds(aligned(base + off, 8), n), :] = out.astype(obuf.dtype)

  def p2_static(j):
    p2(0, j * rows, rows, j % sub_per_seq == 0,
       j % sub_per_seq == sub_per_seq - 1)

  def finish_p2_weights():
    dw_copy.wait()
    w2_copy.wait()
    dw_f32[...] = dw_raw[...].astype(F32)

  w1_copy.wait()
  for c in range(n_pre):
    first, cnt = chunks[c]
    x_chunk(c).wait()
    if c == 1:
      finish_p2_weights()
    if c + LOOKAHEAD < n_chunks:
      x_chunk(c + LOOKAHEAD).start(priority=1)
    for j in range(first, first + cnt):
      p1(0, j * rows)
      if j > 0:
        p2_static(j - 1)
  if n_pre == 1:
    finish_p2_weights()

  if n_iter:
    p2_subs = [[loop_start - 1 + i * per_iter + u for i in range(n_iter)]
               for u in range(per_iter)]
    can_be_first = [any(j % sub_per_seq == 0 for j in js) for js in p2_subs]
    can_be_last = [any(j % sub_per_seq == sub_per_seq - 1 for j in js)
                   for js in p2_subs]

    def body(i, _):
      j0 = loop_start + i * per_iter
      c = n_pre + i
      x_copy(c, j0, per_iter).wait()
      if n_iter > LOOKAHEAD:
        @pl.when(i + LOOKAHEAD < n_iter)
        def _():
          x_copy(c + LOOKAHEAD, j0 + LOOKAHEAD * per_iter,
                 per_iter).start(priority=1)
      if n_iter >= LOOKAHEAD:
        @pl.when(i == n_iter - LOOKAHEAD)
        def _():
          x_chunk(n_chunks - 1).start(priority=1)
      if loop_start > 1:
        @pl.when(i == 0)
        def _():
          out_copy(0, (loop_start - 1) * rows).start(priority=1)
      base = (j0 - 1) * rows
      for u in range(per_iter):
        p1(base, (u + 1) * rows)
        pos = (j0 - 1 + u) % sub_per_seq
        p2(base, u * rows, rows,
           (pos == 0) if can_be_first[u] else False,
           (pos == sub_per_seq - 1) if can_be_last[u] else False)
        out_copy(base + u * rows, rows).start(priority=1)
      return None

    lax.fori_loop(0, n_iter, body, None)
  elif loop_start > 1:
    out_copy(0, (loop_start - 1) * rows).start(priority=1)

  first, cnt = chunks[-1]
  x_chunk(n_chunks - 1).wait()
  for j in range(first, first + cnt - 1):
    p1(0, j * rows)
    p2_static(j - 1)
    out_copy((j - 1) * rows, rows).start(priority=1)
  piece = rows // fine
  row0 = (n_sub - 2) * rows
  for q in range(2 * fine):
    if fine <= q + 1 < 2 * fine:
      p1(0, row0 + (q + 1) * piece, piece)
    off = row0 + q * piece
    p2(0, off, piece, off % seq == 0, (off + piece) % seq == 0)
    out_copy(off, piece).start(priority=1)
  pltpu.make_async_copy(obuf, obuf, o_sem.at[0]).wait()


@jax.jit
def pallas_standalone__conformer_conv_module__speech_kernel(
    x: jax.Array,
    w_pw1: jax.Array,
    dw: jax.Array,
    w_pw2: jax.Array,
):
  batch, seq, dim = x.shape
  taps = dw.shape[0]
  assert dim % LANES == 0 and taps % 2 == 1 and taps // 2 <= 8
  assert w_pw1.shape == (dim, 2 * dim) and w_pw2.shape == (dim, dim)
  rows, pre, per_iter, n_iter, post, fine = _schedule(seq, batch)
  n_tok = batch * seq
  n_chunks = len(pre) + n_iter + 1

  in_hbm = pl.BlockSpec(memory_space=pl.ANY)
  out = pl.pallas_call(
      functools.partial(
          _conformer_conv_kernel, batch=batch, seq=seq, dim=dim, taps=taps,
          rows=rows, pre=pre, per_iter=per_iter, n_iter=n_iter, post=post,
          fine=fine),
      in_specs=[in_hbm] * 4,
      out_specs=in_hbm,
      out_shape=jax.ShapeDtypeStruct((n_tok, dim), x.dtype),
      scratch_shapes=[
          pltpu.VMEM((n_tok, dim), x.dtype),
          pltpu.VMEM((n_tok, dim), x.dtype),
          pltpu.VMEM((dim // LANES, n_tok + 2 * PAD_ROWS, LANES), F32),
          pltpu.VMEM((dim, 2 * dim), w_pw1.dtype),
          pltpu.VMEM((taps, dim), dw.dtype),
          pltpu.VMEM((taps, dim), F32),
          pltpu.VMEM((dim, dim), w_pw2.dtype),
          pltpu.SemaphoreType.DMA((n_chunks,)),
          pltpu.SemaphoreType.DMA((1,)),
          pltpu.SemaphoreType.DMA((3,)),
      ],
      compiler_params=pltpu.CompilerParams(
          vmem_limit_bytes=100 * 1024 * 1024),
  )(x.reshape(n_tok, dim), w_pw1, dw, w_pw2)
  return out.reshape(batch, seq, dim)
```
